```python
import jax
import jax.numpy as jnp

def _softmax(x, axis=-1):
    return jax.nn.softmax(x, axis=axis)

def _gelu(x):
    return jax.nn.gelu(x, approximate=True)

def _silu(x):
    return jax.nn.silu(x)

def _sigmoid(x):
    return jax.nn.sigmoid(x)

def _layernorm(x, axis=-1, eps=1e-05):
    m = jnp.mean(x, axis=axis, keepdims=True)
    v = jnp.var(x, axis=axis, keepdims=True)
    return (x - m) / jnp.sqrt(v + eps)

def _scatter_add(tgt, idx, src, axis=0):
    return tgt.at[idx].add(src)

def _segment_sum(src, seg, n):
    return jax.ops.segment_sum(src, seg, n)

class _Rng:

    def __init__(self, key):
        self._k = key

    def _next(self):
        self._k, sub = jax.random.split(self._k)
        return sub

    def normal(self, shape):
        return jax.random.normal(self._next(), shape, dtype=jnp.bfloat16)

    def randint(self, lo, hi, shape):
        return jax.random.randint(self._next(), shape, lo, hi, dtype=jnp.int32)

    def uniform(self, shape, lo=0.0, hi=1.0):
        return jax.random.uniform(self._next(), shape, jnp.bfloat16, lo, hi)

    def permutation(self, n):
        return jax.random.permutation(self._next(), n)
kernel_name = 'adaLN_cond__sliding_block_cached__moe_arch_mod__decode'

def setup_inputs():
    _rng = _Rng(jax.random.key(int.from_bytes(__import__("os").urandom(4), "little")))
    _w = lambda a: (lambda t: t.astype(jnp.bfloat16) if jnp.issubdtype(t.dtype, jnp.floating) else t)(jnp.asarray(a))

    def _A_setup():
        B, Sq, D = (8, 1, 576)
        Hq, Hkv, Sk, Dh = (32, 16, 8192, 128)
        assert Hq % Hkv == 0, (Hq, Hkv)
        return {'x': _w((lambda *s: _rng.normal(s) * 0.05)(B, Sq, D)), 'k_cache': _w((lambda *s: _rng.normal(s) * 0.05)(B, Hkv, Sk, Dh)), 'v_cache': _w((lambda *s: _rng.normal(s) * 0.05)(B, Hkv, Sk, Dh)), 'wq': _w((lambda *s: _rng.normal(s) * 0.05)(D, Hq * Dh) * D ** (-0.5)), 'wo': _w((lambda *s: _rng.normal(s) * 0.05)(Hq * Dh, D) * (Hq * Dh) ** (-0.5))}
    _A_in = _A_setup()

    def _B_setup():
        B, S, D, F, C = (8, 1, 576, 4608, 1)
        return {'x': _w((lambda *s: _rng.normal(s) * 0.05)(B, S, D)), 'w_r': _w((lambda *s: _rng.normal(s) * 0.05)(D)), 'w_gate': _w((lambda *s: _rng.normal(s) * 0.05)(D, F)), 'w_up': _w((lambda *s: _rng.normal(s) * 0.05)(D, F)), 'w_down': _w((lambda *s: _rng.normal(s) * 0.05)(F, D))}
    _B_in = _B_setup()
    return {'A_x': _A_in['x'], 'A_k_cache': _A_in['k_cache'], 'A_v_cache': _A_in['v_cache'], 'A_wq': _A_in['wq'], 'A_wo': _A_in['wo'], 'B_x': _B_in['x'], 'B_w_r': _B_in['w_r'], 'B_w_gate': _B_in['w_gate'], 'B_w_up': _B_in['w_up'], 'B_w_down': _B_in['w_down'], 'c': _w((lambda *s: _rng.normal(s) * 0.05)(8, 576)), 'w_mod': _w((lambda *s: _rng.normal(s) * 0.05)(576, 6 * 576) * 576 ** (-0.5))}

def reference(A_x, A_k_cache, A_v_cache, A_wq, A_wo, B_x, B_w_r, B_w_gate, B_w_up, B_w_down, c, w_mod):

    def _A_ref(x, k_cache, v_cache, wq, wo):
        B, Sq, D = x.shape
        Hq, Dh = (32, 128)
        Hkv, Sk = (k_cache.shape[1], k_cache.shape[2])
        W = min(4096, max(256, Sk // 4))
        rep = Hq // Hkv
        q = (lambda x, *d: x.transpose(*d))((x @ wq).reshape(B, Sq, Hq, Dh), 0, 2, 1, 3)
        k = jnp.repeat(k_cache[:, :, Sk - W:, :], rep, axis=1)
        v = jnp.repeat(v_cache[:, :, Sk - W:, :], rep, axis=1)
        scores = jnp.einsum('bhqd,bhkd->bhqk', q, k) * Dh ** (-0.5)
        p = _softmax(scores, axis=-1)
        o = jnp.einsum('bhqk,bhkd->bhqd', p, v)
        return (lambda x, *d: x.transpose(*d))(o, 0, 2, 1, 3).reshape(B, Sq, Hq * Dh) @ wo

    def _B_ref(x, w_r, w_gate, w_up, w_down):
        B, S, D = x.shape
        C = 1
        r = x @ w_r
        idx = jnp.argsort(-r, axis=-1)[:, :C]
        idx_e = jnp.repeat(idx.reshape(B, C, 1), D, axis=2)
        x_sel = jnp.take_along_axis(x, idx_e, axis=1)
        g = _silu(x_sel @ w_gate)
        u = x_sel @ w_up
        y = g * u @ w_down
        r_sel = _sigmoid(jnp.take_along_axis(r, idx, axis=1))
        y = y * r_sel.reshape(B, C, 1)
        b_off = (jnp.arange(B) * S).reshape(B, 1)
        flat_idx = (idx + b_off).reshape(B * C)
        zero = (x * 0.0).reshape(B * S, D)
        upd = _scatter_add(zero, flat_idx, y.reshape(B * C, D), axis=0)
        return x + upd.reshape(B, S, D)
    x = A_x
    mod = (_silu(c) @ w_mod).reshape(c.shape[0], 6, 1, -1)
    sa, ca, ga, sb, cb, gb = (mod[:, 0].copy(), mod[:, 1].copy(), mod[:, 2].copy(), mod[:, 3].copy(), mod[:, 4].copy(), mod[:, 5].copy())
    h = _layernorm(x, axis=-1) * (1 + ca) + sa
    x = x + ga * _A_ref(h, A_k_cache, A_v_cache, A_wq, A_wo)
    h = _layernorm(x, axis=-1) * (1 + cb) + sb
    x = x + gb * _B_ref(h, B_w_r, B_w_gate, B_w_up, B_w_down)
    return x
```

```python
import jax
import jax.numpy as jnp
from jax import lax
import jax.experimental.pallas as pl
import jax.experimental.pallas.tpu as pltpu

HQ, DH = 32, 128
BF = jnp.bfloat16
F32 = jnp.float32
NT = (((1,), (1,)), ((), ()))
RG = 8
KV_ROWS = 128
GRP = 512
COLS = 512


def _layernorm(x):
    m = jnp.mean(x, axis=-1, keepdims=True)
    xc = x - m
    v = jnp.mean(xc * xc, axis=-1, keepdims=True)
    return xc / jnp.sqrt(v + 1e-05)


def _kernel(x_hbm, c_hbm, wr_hbm, k_hbm, v_hbm, wq_hbm, wot_hbm, wg_hbm, wu_hbm, wdt_hbm, wmod_hbm,
            o_ref,
            x_v, c_v, wr_v, kv, wq_v, wot_v, wg_v, wu_v, wdt_v, wmod_v,
            mod_v, q_v, s_v, p_v, o_v, g_v, a_v, y_v, kvsem, wsem, dsem):
    B, D = x_hbm.shape
    _, HKV, SK, _ = k_hbm.shape
    W = kv.shape[1]
    REP = HQ // HKV
    M = REP * B
    HALF = D // RG // 2
    NGRP = W // GRP
    PPG = W // (2 * KV_ROWS) // NGRP

    def kv_pair(src, b, h, slot, j):
        for p in range(2):
            r0 = p * (W // 2) + j * KV_ROWS
            pltpu.make_async_copy(src.at[b, h, pl.ds(SK - W + r0, KV_ROWS), :],
                                  kv.at[slot, pl.ds(r0, KV_ROWS), :], kvsem.at[slot]).start(priority=p)

    def wait_all(dst, sem):
        pltpu.make_async_copy(dst, dst, sem).wait()

    def w_rows(src, dst, sem, r, half=HALF):
        n = src.shape[1]
        n0 = (n // 128 + 1) // 2 * 128
        for c0, cn in ((0, n0), (n0, n - n0)):
            for p in range(2):
                rows = pl.ds(pl.multiple_of((r + p * half) * RG, RG), RG)
                pltpu.make_async_copy(src.at[rows, pl.ds(c0, cn)], dst.at[rows, pl.ds(c0, cn)],
                                      sem).start(priority=p)

    def w_issue(src, dst, sem, lo, hi):
        def body(r, _):
            w_rows(src, dst, sem, r)
        lax.fori_loop(lo, hi, body, None)

    def wd_rows(i):
        s = i // 8
        w_rows(wdt_hbm, wdt_v, dsem.at[s], s * 16 + i % 8, jnp.where(s == 4, 4, 8))

    def col_block(i, n):
        return pl.ds(pl.multiple_of(i * n, 128), n)

    def mod_part(i):
        lo = i * D // 128 * 128
        hi = -(-(i + 1) * D // 128) * 128
        return mod_v[:, lo:hi][:, i * D - lo:(i + 1) * D - lo]

    small = [pltpu.make_async_copy(c_hbm, c_v, wsem.at[0]),
             pltpu.make_async_copy(x_hbm, x_v, wsem.at[1]),
             pltpu.make_async_copy(wr_hbm, wr_v, wsem.at[2])]
    for d in small:
        d.start()
    w_issue(wmod_hbm, wmod_v, wsem.at[3], 0, HALF)
    w_issue(wq_hbm, wq_v, wsem.at[4], 0, 18)
    for d in small:
        d.wait()
    cc = c_v[...].astype(F32)
    c_act = (cc * jax.nn.sigmoid(cc)).astype(BF)
    wait_all(wmod_v, wsem.at[3])

    def mod_body(i, _):
        for t in range(2):
            w_rows(wq_hbm, wq_v, wsem.at[4], 18 + 2 * i + t)
        cols = col_block(i, 384)
        mod_v[:, cols] = jnp.dot(c_act, wmod_v[:, cols], preferred_element_type=F32)
    lax.fori_loop(0, 9, mod_body, None)

    def k0_body(b, _):
        for j in range(NGRP * PPG):
            kv_pair(k_hbm, b, 0, b, j)
    lax.fori_loop(0, B // 2, k0_body, None)
    hb = (_layernorm(x_v[...].astype(F32)) * (1 + mod_part(1)) + mod_part(0)).astype(BF)
    s_v[...] = jnp.zeros(s_v.shape, F32)
    wait_all(wq_v, wsem.at[4])

    def q_body(i, _):
        b = B // 2 + i // 2
        for j in range(4):
            kv_pair(k_hbm, b, 0, b, (i % 2) * 4 + j)
        q = jnp.dot(hb, wq_v[:, col_block(i, COLS)], preferred_element_type=F32)
        for j in range(4):
            q_v[2 * i + j // REP, pl.ds((j % REP) * B, B), :] = q[:, j * DH:(j + 1) * DH]
    lax.fori_loop(0, HQ * DH // COLS, q_body, None)

    def head_body(h, _):
        def qk_body(b, _):
            qq = q_v[h].astype(BF)
            mine = lax.broadcasted_iota(jnp.int32, (M, GRP), 0) % B == b
            wait_all(kv.at[b], kvsem.at[b])
            for g in range(NGRP):
                for j in range(PPG):
                    kv_pair(v_hbm, b, h, B + b, g * PPG + j)
                keys = pl.ds(g * GRP, GRP)
                s = lax.dot_general(qq, kv[b, keys, :], NT, preferred_element_type=F32)
                s_v[:, keys] = jnp.where(mine, s, s_v[:, keys])
        lax.fori_loop(0, B, qk_body, None)

        s = s_v[...] * (DH ** -0.5)
        m = jnp.max(s, axis=-1, keepdims=True)
        p = jnp.exp(s - m)
        l = jnp.sum(p, axis=-1, keepdims=True)
        p_v[...] = p.astype(BF)

        def pv_loop(issue):
            def pv_body(b, o):
                mine = lax.broadcasted_iota(jnp.int32, (M, DH), 0) % B == b
                wait_all(kv.at[B + b], kvsem.at[B + b])
                acc = None
                for g in range(NGRP):
                    issue(b, g)
                    keys = pl.ds(g * GRP, GRP)
                    t = jnp.dot(p_v[:, keys], kv[B + b, keys, :], preferred_element_type=F32)
                    acc = t if acc is None else acc + t
                return jnp.where(mine, acc, o)
            o = lax.fori_loop(0, B, pv_body, jnp.zeros((M, DH), F32)) / l
            for j in range(REP):
                o_v[REP * h + j] = o[j * B:(j + 1) * B]

        def issue_k(b, g):
            for j in range(PPG):
                kv_pair(k_hbm, b, h + 1, b, g * PPG + j)

        def issue_wo(b, g):
            w_rows(wot_hbm, wot_v, wsem.at[5], b * NGRP + g)

        @pl.when(h < HKV - 1)
        def _():
            pv_loop(issue_k)

        @pl.when(h == HKV - 1)
        def _():
            pv_loop(issue_wo)
    lax.fori_loop(0, HKV, head_body, None)

    w_issue(wot_hbm, wot_v, wsem.at[5], B * NGRP, HALF)
    w_issue(wg_hbm, wg_v, wsem.at[6], 0, 20)
    wait_all(wot_v, wsem.at[5])

    def wo_body(i, att):
        for t in range(2):
            w_rows(wg_hbm, wg_v, wsem.at[6], 20 + 2 * i + t)
        oo = jnp.concatenate([o_v[4 * i + j] for j in range(4)], axis=1).astype(BF)
        return att + lax.dot_general(oo, wot_v[:, col_block(i, COLS)], NT, preferred_element_type=F32)
    att = lax.fori_loop(0, HQ * DH // COLS, wo_body, jnp.zeros((B, D), F32))

    w_issue(wu_hbm, wu_v, wsem.at[7], 0, 18)
    x1 = x_v[...].astype(F32) + mod_part(2) * att
    h2 = _layernorm(x1) * (1 + mod_part(4)) + mod_part(3)
    h2b = h2.astype(BF)
    r = jnp.sum(h2b.astype(F32) * wr_v[...].astype(F32).reshape(1, D), axis=-1, keepdims=True)
    wait_all(wg_v, wsem.at[6])

    def gate_body(i, _):
        for t in range(2):
            w_rows(wu_hbm, wu_v, wsem.at[7], 18 + 2 * i + t)
        cols = col_block(i, COLS)
        g = jnp.dot(h2b, wg_v[:, cols], preferred_element_type=F32)
        g_v[:, cols] = g * jax.nn.sigmoid(g)
    lax.fori_loop(0, 9, gate_body, None)

    def wd_body(i, _):
        wd_rows(i)
    lax.fori_loop(0, 18, wd_body, None)
    wait_all(wu_v, wsem.at[7])

    def up_body(i, _):
        for t in range(2):
            wd_rows(18 + 2 * i + t)
        cols = col_block(i, COLS)
        a_v[:, cols] = g_v[:, cols] * jnp.dot(h2b, wu_v[:, cols], preferred_element_type=F32)
    lax.fori_loop(0, 9, up_body, None)
    a = a_v[...].astype(BF)

    def down_body(s, _):
        rows = col_block(s, 128)
        wait_all(wdt_v.at[rows, :], dsem.at[s])
        y_v[:, rows] = lax.dot_general(a, wdt_v[rows, :], NT, preferred_element_type=F32)
    lax.fori_loop(0, 4, down_body, None)
    wait_all(wdt_v.at[pl.ds(512, D - 512), :], dsem.at[4])
    y_last = lax.dot_general(a, wdt_v[512:D, :], NT, preferred_element_type=F32)
    y = jnp.concatenate([y_v[...], y_last], axis=1) * jax.nn.sigmoid(r)
    o_ref[...] = (x1 + mod_part(5) * (h2 + (h2 * 0.0 + y))).astype(o_ref.dtype)


@jax.jit
def pallas_adaLN_cond__sliding_block_cached__moe_arch_mod__decode_kernel(
    A_x: jax.Array,
    A_k_cache: jax.Array,
    A_v_cache: jax.Array,
    A_wq: jax.Array,
    A_wo: jax.Array,
    B_x: jax.Array,
    B_w_r: jax.Array,
    B_w_gate: jax.Array,
    B_w_up: jax.Array,
    B_w_down: jax.Array,
    c: jax.Array,
    w_mod: jax.Array,
):
    del B_x
    B, S, D = A_x.shape
    HKV, SK = A_k_cache.shape[1], A_k_cache.shape[2]
    F = B_w_gate.shape[1]
    W = min(4096, max(256, SK // 4))
    M = HQ // HKV * B
    assert (B, S, D, HKV, W, F) == (8, 1, 576, 16, 2048, 4608)

    hbm = pl.BlockSpec(memory_space=pltpu.HBM)
    out = pl.pallas_call(
        _kernel,
        out_shape=jax.ShapeDtypeStruct((B, D), A_x.dtype),
        in_specs=[hbm] * 11,
        out_specs=pl.BlockSpec(memory_space=pltpu.VMEM),
        scratch_shapes=[
            pltpu.VMEM((B, D), BF), pltpu.VMEM((B, D), BF), pltpu.VMEM((D,), BF),
            pltpu.VMEM((2 * B, W, DH), BF),
            pltpu.VMEM((D, HQ * DH), BF), pltpu.VMEM((D, HQ * DH), BF),
            pltpu.VMEM((D, F), BF), pltpu.VMEM((D, F), BF), pltpu.VMEM((D, F), BF),
            pltpu.VMEM((D, 6 * D), BF),
            pltpu.VMEM((B, 6 * D), F32), pltpu.VMEM((HKV, M, DH), F32),
            pltpu.VMEM((M, W), F32), pltpu.VMEM((M, W), BF),
            pltpu.VMEM((HQ, B, DH), F32), pltpu.VMEM((B, F), F32), pltpu.VMEM((B, F), F32),
            pltpu.VMEM((B, 512), F32),
            pltpu.SemaphoreType.DMA((2 * B,)), pltpu.SemaphoreType.DMA((8,)), pltpu.SemaphoreType.DMA((5,)),
        ],
        compiler_params=pltpu.CompilerParams(vmem_limit_bytes=64 * 1024 * 1024),
    )(A_x.reshape(B, D), c, B_w_r, A_k_cache, A_v_cache, A_wq, A_wo.T, B_w_gate, B_w_up, B_w_down.T, w_mod)
    return out.reshape(B, S, D)
```

```python
import jax
import jax.numpy as jnp
from jax import lax
import jax.experimental.pallas as pl
import jax.experimental.pallas.tpu as pltpu

HQ, DH = 32, 128
BF = jnp.bfloat16
F32 = jnp.float32
NT = (((1,), (1,)), ((), ()))
RG = 8
KV_COPIES = 6
COLS = 512


def _layernorm(x):
    m = jnp.mean(x, axis=-1, keepdims=True)
    xc = x - m
    v = jnp.mean(xc * xc, axis=-1, keepdims=True)
    return xc / jnp.sqrt(v + 1e-05)


def _split(start, size, parts, unit):
    edges = [start + unit * (i * (size // unit) // parts) for i in range(parts + 1)]
    return [(a, b - a) for a, b in zip(edges, edges[1:])]


def _kernel(x_hbm, c_hbm, wr_hbm, k_hbm, v_hbm, wq_hbm, wot_hbm, wg_hbm, wu_hbm, wdt_hbm, wmod_hbm,
            o_ref,
            x_v, c_v, wr_v, k_v, v_v, wq_v, wot_v, wg_v, wu_v, wdt_v, wmod_v,
            mod_v, q_v, s_v, p_v, o_v, g_v, a_v, base_v, scale_v, ksem, vsem, wsem, dsem):
    B, D = x_hbm.shape
    _, HKV, SK, _ = k_hbm.shape
    F = wg_hbm.shape[1]
    W = k_v.shape[1]
    REP = HQ // HKV
    M = REP * B
    HALF = D // RG // 2
    SLAB = 128
    DLO = D // SLAB * SLAB

    def wait_all(dst, sem):
        pltpu.make_async_copy(dst, dst, sem).wait()

    def kv_start(src, dst, sem, b, h):
        for pair in zip(_split(0, W // 2, KV_COPIES, RG), _split(W // 2, W // 2, KV_COPIES, RG)):
            for prio, (r0, n) in enumerate(pair):
                pltpu.make_async_copy(src.at[b, h, pl.ds(SK - W + r0, n), :],
                                      dst.at[b, pl.ds(r0, n), :], sem.at[b]).start(priority=prio)

    def w_copy(src, dst, sem, r, cols, prio):
        rows = pl.ds(pl.multiple_of(r * RG, RG), RG)
        pltpu.make_async_copy(src.at[rows, pl.ds(*cols)], dst.at[rows, pl.ds(*cols)],
                              sem).start(priority=prio)

    def w_rows(src, dst, sem, r):
        for cols in _split(0, src.shape[1], 2, 128):
            w_copy(src, dst, sem, r, cols, 0)
            w_copy(src, dst, sem, r + HALF, cols, 1)

    def w_issue(src, dst, sem, lo, hi):
        lax.fori_loop(lo, hi, lambda r, _: w_rows(src, dst, sem, r), None)

    def wd_rows(r):
        for cols in _split(0, F, 2, 128):
            w_copy(wdt_hbm, wdt_v, dsem.at[r // (SLAB // RG)], r, cols, 0)
            w_copy(wdt_hbm, wdt_v, dsem.at[(r + HALF) // (SLAB // RG)], r + HALF, cols, 1)

    def col_block(i, n):
        return pl.ds(pl.multiple_of(i * n, 128), n)

    def mod_part(i):
        lo = i * D // 128 * 128
        hi = -(-(i + 1) * D // 128) * 128
        return mod_v[:, lo:hi][:, i * D - lo:(i + 1) * D - lo]

    small = [pltpu.make_async_copy(c_hbm, c_v, wsem.at[0]),
             pltpu.make_async_copy(x_hbm, x_v, wsem.at[0]),
             pltpu.make_async_copy(wr_hbm, wr_v, wsem.at[0])]
    for d in small:
        d.start()
    w_issue(wmod_hbm, wmod_v, wsem.at[1], 0, HALF)
    w_issue(wq_hbm, wq_v, wsem.at[2], 0, 18)
    for d in small:
        d.wait()
    cc = c_v[...].astype(F32)
    c_act = (cc * jax.nn.sigmoid(cc)).astype(BF)
    wait_all(wmod_v, wsem.at[1])

    def mod_body(i, _):
        for t in range(2):
            w_rows(wq_hbm, wq_v, wsem.at[2], 18 + 2 * i + t)
        cols = col_block(i, 6 * D // 9)
        mod_v[:, cols] = jnp.dot(c_act, wmod_v[:, cols], preferred_element_type=F32)
    lax.fori_loop(0, 9, mod_body, None)

    lax.fori_loop(0, B - 2, lambda b, _: kv_start(k_hbm, k_v, ksem, b, 0), None)
    hb = (_layernorm(x_v[...].astype(F32)) * (1 + mod_part(1)) + mod_part(0)).astype(BF)
    s_v[...] = jnp.zeros(s_v.shape, F32)
    wait_all(wq_v, wsem.at[2])
    lax.fori_loop(B - 2, B, lambda b, _: kv_start(k_hbm, k_v, ksem, b, 0), None)

    def q_body(i, _):
        q = jnp.dot(hb, wq_v[:, col_block(i, COLS)], preferred_element_type=F32)
        for j in range(COLS // DH):
            q_v[COLS // DH // REP * i + j // REP, pl.ds(j % REP * B, B), :] = q[:, j * DH:(j + 1) * DH]
    lax.fori_loop(0, HQ * DH // COLS, q_body, None)

    def head_body(h, _):
        def qk_body(b, _):
            mine = lax.broadcasted_iota(jnp.int32, (M, W), 0) % B == b
            wait_all(k_v.at[b], ksem.at[b])
            kv_start(v_hbm, v_v, vsem, b, h)
            s = lax.dot_general(q_v[h].astype(BF), k_v[b], NT, preferred_element_type=F32)
            s_v[...] = jnp.where(mine, s, s_v[...])
        lax.fori_loop(0, B, qk_body, None)

        s = s_v[...] * (DH ** -0.5)
        p = jnp.exp(s - jnp.max(s, axis=-1, keepdims=True))
        l = jnp.sum(p, axis=-1, keepdims=True)
        p_v[...] = p.astype(BF)

        def pv_body(b, o):
            mine = lax.broadcasted_iota(jnp.int32, (M, DH), 0) % B == b
            wait_all(v_v.at[b], vsem.at[b])

            @pl.when(h < HKV - 1)
            def _():
                kv_start(k_hbm, k_v, ksem, b, h + 1)

            @pl.when(h == HKV - 1)
            def _():
                w_issue(wot_hbm, wot_v, wsem.at[3], 4 * b, 4 * b + 4)
            return jnp.where(mine, jnp.dot(p_v[...], v_v[b], preferred_element_type=F32), o)
        o = lax.fori_loop(0, B, pv_body, jnp.zeros((M, DH), F32)) / l
        for j in range(REP):
            o_v[REP * h + j] = o[j * B:(j + 1) * B]
    lax.fori_loop(0, HKV, head_body, None)

    w_issue(wot_hbm, wot_v, wsem.at[3], 4 * B, HALF)
    w_issue(wg_hbm, wg_v, wsem.at[4], 0, 20)
    wait_all(wot_v, wsem.at[3])

    def wo_body(i, att):
        for t in range(2):
            w_rows(wg_hbm, wg_v, wsem.at[4], 20 + 2 * i + t)
        heads = [o_v[COLS // DH * i + j] for j in range(COLS // DH)]
        return att + lax.dot_general(jnp.concatenate(heads, axis=1).astype(BF),
                                     wot_v[:, col_block(i, COLS)], NT, preferred_element_type=F32)
    att = lax.fori_loop(0, HQ * DH // COLS, wo_body, jnp.zeros((B, D), F32))

    w_issue(wu_hbm, wu_v, wsem.at[5], 0, 18)
    x1 = x_v[...].astype(F32) + mod_part(2) * att
    h2 = _layernorm(x1) * (1 + mod_part(4)) + mod_part(3)
    h2b = h2.astype(BF)
    r = jnp.sum(h2b.astype(F32) * wr_v[...].astype(F32).reshape(1, D), axis=-1, keepdims=True)
    gb = mod_part(5)
    base_v[...] = x1 + gb * (h2 + h2 * 0.0)
    scale_v[...] = gb * jax.nn.sigmoid(r)
    wait_all(wg_v, wsem.at[4])

    def gate_body(i, _):
        for t in range(2):
            w_rows(wu_hbm, wu_v, wsem.at[5], 18 + 2 * i + t)
        cols = col_block(i, COLS)
        g = jnp.dot(h2b, wg_v[:, cols], preferred_element_type=F32)
        g_v[:, cols] = g * jax.nn.sigmoid(g)
    lax.fori_loop(0, F // COLS, gate_body, None)

    lax.fori_loop(0, 19, lambda i, _: wd_rows(i), None)
    wait_all(wu_v, wsem.at[5])

    def up_body(i, _):
        wd_rows(19 + i)
        cols = col_block(i, COLS)
        a_v[:, cols] = g_v[:, cols] * jnp.dot(h2b, wu_v[:, cols], preferred_element_type=F32)
    lax.fori_loop(0, F // COLS, up_body, None)

    for i, cols in enumerate(_split(0, F, 2, 128)):
        def last_rows(r, _, i=i, cols=cols):
            w_copy(wdt_hbm, wdt_v, dsem.at[r // (SLAB // RG)], r, cols, 0)
            w_copy(wdt_hbm, wdt_v, dsem.at[DLO // SLAB + i], r + HALF, cols, 1)
        lax.fori_loop(DLO // RG - HALF, HALF, last_rows, None)

    def down_body(i, _):
        rows = col_block(i, SLAB)
        a = a_v[...].astype(BF)
        wait_all(wdt_v.at[rows, :], dsem.at[i])
        y = lax.dot_general(a, wdt_v[rows, :], NT, preferred_element_type=F32)
        o_ref[:, rows] = (base_v[:, rows] + scale_v[:, rows] * y).astype(o_ref.dtype)
    lax.fori_loop(0, DLO // SLAB, down_body, None)

    y = jnp.zeros((B, D - DLO), F32)
    for i, cols in enumerate(_split(0, F, 2, 128)):
        a = a_v[:, pl.ds(*cols)].astype(BF)
        wait_all(wdt_v.at[pl.ds(DLO, D - DLO), pl.ds(*cols)], dsem.at[DLO // SLAB + i])
        y = y + lax.dot_general(a, wdt_v[DLO:D, pl.ds(*cols)], NT, preferred_element_type=F32)
    o_ref[:, DLO:D] = (base_v[:, DLO:D] + scale_v[:, DLO:D] * y).astype(o_ref.dtype)


@jax.jit
def pallas_adaLN_cond__sliding_block_cached__moe_arch_mod__decode_kernel(
    A_x: jax.Array,
    A_k_cache: jax.Array,
    A_v_cache: jax.Array,
    A_wq: jax.Array,
    A_wo: jax.Array,
    B_x: jax.Array,
    B_w_r: jax.Array,
    B_w_gate: jax.Array,
    B_w_up: jax.Array,
    B_w_down: jax.Array,
    c: jax.Array,
    w_mod: jax.Array,
):
    del B_x
    B, S, D = A_x.shape
    HKV, SK = A_k_cache.shape[1], A_k_cache.shape[2]
    F = B_w_gate.shape[1]
    W = min(4096, max(256, SK // 4))
    M = HQ // HKV * B
    assert (B, S, D, HKV, W, F) == (8, 1, 576, 16, 2048, 4608)

    hbm = pl.BlockSpec(memory_space=pltpu.HBM)
    out = pl.pallas_call(
        _kernel,
        out_shape=jax.ShapeDtypeStruct((B, D), A_x.dtype),
        in_specs=[hbm] * 11,
        out_specs=pl.BlockSpec(memory_space=pltpu.VMEM),
        scratch_shapes=[
            pltpu.VMEM((B, D), BF), pltpu.VMEM((B, D), BF), pltpu.VMEM((D,), BF),
            pltpu.VMEM((B, W, DH), BF), pltpu.VMEM((B, W, DH), BF),
            pltpu.VMEM((D, HQ * DH), BF), pltpu.VMEM((D, HQ * DH), BF),
            pltpu.VMEM((D, F), BF), pltpu.VMEM((D, F), BF), pltpu.VMEM((D, F), BF),
            pltpu.VMEM((D, 6 * D), BF),
            pltpu.VMEM((B, 6 * D), F32), pltpu.VMEM((HKV, M, DH), F32),
            pltpu.VMEM((M, W), F32), pltpu.VMEM((M, W), BF),
            pltpu.VMEM((HQ, B, DH), F32), pltpu.VMEM((B, F), F32), pltpu.VMEM((B, F), F32),
            pltpu.VMEM((B, D), F32), pltpu.VMEM((B, D), F32),
            pltpu.SemaphoreType.DMA((B,)), pltpu.SemaphoreType.DMA((B,)),
            pltpu.SemaphoreType.DMA((6,)), pltpu.SemaphoreType.DMA((6,)),
        ],
        compiler_params=pltpu.CompilerParams(
            vmem_limit_bytes=64 * 1024 * 1024,
            disable_bounds_checks=True,
            disable_semaphore_checks=True,
        ),
    )(A_x.reshape(B, D), c, B_w_r, A_k_cache, A_v_cache, A_wq, A_wo.T, B_w_gate, B_w_up, B_w_down.T, w_mod)
    return out.reshape(B, S, D)
```

```python
import jax
import jax.numpy as jnp
from jax import lax
import jax.experimental.pallas as pl
import jax.experimental.pallas.tpu as pltpu

HQ, DH = 32, 128
BF = jnp.bfloat16
F32 = jnp.float32
NT = (((1,), (1,)), ((), ()))
RG = 8
COLS = 512
KV_ROWS = ((200, 184, 120, 184, 160, 184), (160, 168, 160, 176, 200, 152))


def _layernorm(x):
    m = jnp.mean(x, axis=-1, keepdims=True)
    xc = x - m
    v = jnp.mean(xc * xc, axis=-1, keepdims=True)
    return xc / jnp.sqrt(v + 1e-05)


def _col_halves(n):
    left = n // 128 // 2 * 128
    return (0, left), (left, n - left)


def _kernel(x_hbm, c_hbm, wr_hbm, k_hbm, v_hbm, wq_hbm, wot_hbm, wg_hbm, wu_hbm, wdt_hbm, wmod_hbm,
            o_ref,
            x_v, c_v, wr_v, k_v, v_v, wq_v, wot_v, wg_v, wu_v, wdt_v, wmod_v,
            mod_v, q_v, s_v, p_v, o_v, g_v, a_v, base_v, scale_v, ksem, vsem, wsem, dsem):
    B, D = x_hbm.shape
    _, HKV, SK, _ = k_hbm.shape
    F = wg_hbm.shape[1]
    W = k_v.shape[1]
    REP = HQ // HKV
    M = REP * B
    HALF = D // RG // 2
    SLAB = 128

    def wait_all(dst, sem):
        pltpu.make_async_copy(dst, dst, sem).wait()

    def kv_start(src, dst, sem, b, h):
        r0 = [0, sum(KV_ROWS[0])]
        for pair in zip(*KV_ROWS):
            for prio, n in enumerate(pair):
                pltpu.make_async_copy(src.at[b, h, pl.ds(SK - W + r0[prio], n), :],
                                      dst.at[b, pl.ds(r0[prio], n), :], sem.at[b]).start(priority=prio)
                r0[prio] += n

    def w_copy(src, dst, sem, r, cols, prio):
        rows = pl.ds(pl.multiple_of(r * RG, RG), RG)
        pltpu.make_async_copy(src.at[rows, pl.ds(*cols)], dst.at[rows, pl.ds(*cols)],
                              sem).start(priority=prio)

    def w_rows(src, dst, sem, r):
        for cols in _col_halves(src.shape[1]):
            w_copy(src, dst, sem, r, cols, 0)
            w_copy(src, dst, sem, r + HALF, cols, 1)

    def w_issue(src, dst, sem, lo, hi):
        lax.fori_loop(lo, hi, lambda r, _: w_rows(src, dst, sem, r), None)

    def wd_rows(r):
        for cols in _col_halves(F):
            w_copy(wdt_hbm, wdt_v, dsem.at[r // (SLAB // RG)], r, cols, 0)
            w_copy(wdt_hbm, wdt_v, dsem.at[(r + HALF) // (SLAB // RG)], r + HALF, cols, 1)

    def col_block(i, n):
        return pl.ds(pl.multiple_of(i * n, 128), n)

    def mod_part(i):
        lo = i * D // 128 * 128
        hi = -(-(i + 1) * D // 128) * 128
        return mod_v[:, lo:hi][:, i * D - lo:(i + 1) * D - lo]

    small = [pltpu.make_async_copy(c_hbm, c_v, wsem.at[0]),
             pltpu.make_async_copy(x_hbm, x_v, wsem.at[0]),
             pltpu.make_async_copy(wr_hbm, wr_v, wsem.at[0])]

    def prime(r, _):
        for rg in (r, r + HALF):
            for cols in _col_halves(6 * D):
                w_copy(wmod_hbm, wmod_v, wsem.at[1], rg, cols, 1)
    lax.fori_loop(0, 8, prime, None)
    for d in small:
        d.start()
    w_issue(wmod_hbm, wmod_v, wsem.at[1], 8, HALF)
    w_issue(wq_hbm, wq_v, wsem.at[2], 0, 18)
    for d in small:
        d.wait()
    cc = c_v[...].astype(F32)
    c_act = (cc * jax.nn.sigmoid(cc)).astype(BF)
    wait_all(wmod_v, wsem.at[1])

    def mod_body(i, _):
        for t in range(2):
            w_rows(wq_hbm, wq_v, wsem.at[2], 18 + 2 * i + t)
        cols = col_block(i, 6 * D // 9)
        mod_v[:, cols] = jnp.dot(c_act, wmod_v[:, cols], preferred_element_type=F32)
    lax.fori_loop(0, 9, mod_body, None)

    lax.fori_loop(0, B - 2, lambda b, _: kv_start(k_hbm, k_v, ksem, b, 0), None)
    hb = (_layernorm(x_v[...].astype(F32)) * (1 + mod_part(1)) + mod_part(0)).astype(BF)
    s_v[...] = jnp.zeros(s_v.shape, F32)
    wait_all(wq_v, wsem.at[2])
    lax.fori_loop(B - 2, B, lambda b, _: kv_start(k_hbm, k_v, ksem, b, 0), None)

    def q_body(i, _):
        q = jnp.dot(hb, wq_v[:, col_block(i, COLS)], preferred_element_type=F32)
        for j in range(COLS // DH):
            q_v[COLS // DH // REP * i + j // REP, pl.ds(j % REP * B, B), :] = q[:, j * DH:(j + 1) * DH]
    lax.fori_loop(0, HQ * DH // COLS, q_body, None)

    def head_body(h, _):
        def qk_body(b, _):
            mine = lax.broadcasted_iota(jnp.int32, (M, W), 0) % B == b
            wait_all(k_v.at[b], ksem.at[b])
            kv_start(v_hbm, v_v, vsem, b, h)
            s = lax.dot_general(q_v[h].astype(BF), k_v[b], NT, preferred_element_type=F32)
            s_v[...] = jnp.where(mine, s, s_v[...])
        lax.fori_loop(0, B, qk_body, None)

        s = s_v[...] * (DH ** -0.5)
        p = jnp.exp(s - jnp.max(s, axis=-1, keepdims=True))
        l = jnp.sum(p, axis=-1, keepdims=True)
        p_v[...] = p.astype(BF)

        def pv_body(b, o):
            mine = lax.broadcasted_iota(jnp.int32, (M, DH), 0) % B == b
            wait_all(v_v.at[b], vsem.at[b])

            @pl.when(h < HKV - 1)
            def _():
                kv_start(k_hbm, k_v, ksem, b, h + 1)

            @pl.when(h == HKV - 1)
            def _():
                w_issue(wot_hbm, wot_v, wsem.at[3], 4 * b, 4 * b + 4)
            return jnp.where(mine, jnp.dot(p_v[...], v_v[b], preferred_element_type=F32), o)
        o = lax.fori_loop(0, B, pv_body, jnp.zeros((M, DH), F32)) / l
        for j in range(REP):
            o_v[REP * h + j] = o[j * B:(j + 1) * B]
    lax.fori_loop(0, HKV, head_body, None)

    w_issue(wot_hbm, wot_v, wsem.at[3], 4 * B, HALF)
    w_issue(wg_hbm, wg_v, wsem.at[4], 0, 20)
    wait_all(wot_v, wsem.at[3])

    def wo_body(i, att):
        for t in range(2):
            w_rows(wg_hbm, wg_v, wsem.at[4], 20 + 2 * i + t)
        heads = [o_v[COLS // DH * i + j] for j in range(COLS // DH)]
        return att + lax.dot_general(jnp.concatenate(heads, axis=1).astype(BF),
                                     wot_v[:, col_block(i, COLS)], NT, preferred_element_type=F32)
    att = lax.fori_loop(0, HQ * DH // COLS, wo_body, jnp.zeros((B, D), F32))

    w_issue(wu_hbm, wu_v, wsem.at[5], 0, 18)
    x1 = x_v[...].astype(F32) + mod_part(2) * att
    h2 = _layernorm(x1) * (1 + mod_part(4)) + mod_part(3)
    h2b = h2.astype(BF)
    r = jnp.sum(h2b.astype(F32) * wr_v[...].astype(F32).reshape(1, D), axis=-1, keepdims=True)
    gb = mod_part(5)
    base_v[...] = x1 + gb * (h2 + h2 * 0.0)
    scale_v[...] = gb * jax.nn.sigmoid(r)
    wait_all(wg_v, wsem.at[4])

    def gate_body(i, _):
        for t in range(2):
            w_rows(wu_hbm, wu_v, wsem.at[5], 18 + 2 * i + t)
        cols = col_block(i, COLS)
        g = jnp.dot(h2b, wg_v[:, cols], preferred_element_type=F32)
        g_v[:, cols] = g * jax.nn.sigmoid(g)
    lax.fori_loop(0, F // COLS, gate_body, None)

    lax.fori_loop(0, 19, lambda i, _: wd_rows(i), None)
    wait_all(wu_v, wsem.at[5])

    def up_body(i, _):
        wd_rows(19 + i)
        cols = col_block(i, COLS)
        a_v[:, cols] = g_v[:, cols] * jnp.dot(h2b, wu_v[:, cols], preferred_element_type=F32)
    lax.fori_loop(0, F // COLS, up_body, None)

    lax.fori_loop(19 + F // COLS, HALF, lambda i, _: wd_rows(i), None)

    def down(i, cols):
        a = a_v[...].astype(BF)
        wait_all(wdt_v.at[cols, :], dsem.at[i])
        y = lax.dot_general(a, wdt_v[cols, :], NT, preferred_element_type=F32)
        o_ref[:, cols] = (base_v[:, cols] + scale_v[:, cols] * y).astype(o_ref.dtype)
    lax.fori_loop(0, D // SLAB, lambda i, _: down(i, col_block(i, SLAB)), None)
    down(D // SLAB, pl.ds(D // SLAB * SLAB, D % SLAB))


@jax.jit
def pallas_adaLN_cond__sliding_block_cached__moe_arch_mod__decode_kernel(
    A_x: jax.Array,
    A_k_cache: jax.Array,
    A_v_cache: jax.Array,
    A_wq: jax.Array,
    A_wo: jax.Array,
    B_x: jax.Array,
    B_w_r: jax.Array,
    B_w_gate: jax.Array,
    B_w_up: jax.Array,
    B_w_down: jax.Array,
    c: jax.Array,
    w_mod: jax.Array,
):
    del B_x
    B, S, D = A_x.shape
    HKV, SK = A_k_cache.shape[1], A_k_cache.shape[2]
    F = B_w_gate.shape[1]
    W = min(4096, max(256, SK // 4))
    M = HQ // HKV * B
    assert (B, S, D, HKV, W, F) == (8, 1, 576, 16, 2048, 4608) and sum(map(sum, KV_ROWS)) == W

    hbm = pl.BlockSpec(memory_space=pltpu.HBM)
    out = pl.pallas_call(
        _kernel,
        out_shape=jax.ShapeDtypeStruct((B, D), A_x.dtype),
        in_specs=[hbm] * 11,
        out_specs=pl.BlockSpec(memory_space=pltpu.VMEM),
        scratch_shapes=[
            pltpu.VMEM((B, D), BF), pltpu.VMEM((B, D), BF), pltpu.VMEM((D,), BF),
            pltpu.VMEM((B, W, DH), BF), pltpu.VMEM((B, W, DH), BF),
            pltpu.VMEM((D, HQ * DH), BF), pltpu.VMEM((D, HQ * DH), BF),
            pltpu.VMEM((D, F), BF), pltpu.VMEM((D, F), BF), pltpu.VMEM((D, F), BF),
            pltpu.VMEM((D, 6 * D), BF),
            pltpu.VMEM((B, 6 * D), F32), pltpu.VMEM((HKV, M, DH), F32),
            pltpu.VMEM((M, W), F32), pltpu.VMEM((M, W), BF),
            pltpu.VMEM((HQ, B, DH), F32), pltpu.VMEM((B, F), F32), pltpu.VMEM((B, F), F32),
            pltpu.VMEM((B, D), F32), pltpu.VMEM((B, D), F32),
            pltpu.SemaphoreType.DMA((B,)), pltpu.SemaphoreType.DMA((B,)),
            pltpu.SemaphoreType.DMA((6,)), pltpu.SemaphoreType.DMA((5,)),
        ],
        compiler_params=pltpu.CompilerParams(
            vmem_limit_bytes=64 * 1024 * 1024,
            disable_semaphore_checks=True,
        ),
    )(A_x.reshape(B, D), c, B_w_r, A_k_cache, A_v_cache, A_wq, A_wo.T, B_w_gate, B_w_up, B_w_down.T, w_mod)
    return out.reshape(B, S, D)
```
